```python
import os as _os
_os.environ.setdefault("JAX_PLATFORMS", "cpu")
import jax
import jax.numpy as jnp

def _softmax(x, axis=-1):
    return jax.nn.softmax(x, axis=axis)
def _gelu(x):
    return jax.nn.gelu(x, approximate=True)
def _silu(x):
    return jax.nn.silu(x)
def _sigmoid(x):
    return jax.nn.sigmoid(x)
def _layernorm(x, axis=-1, eps=1e-5):
    m = jnp.mean(x, axis=axis, keepdims=True)
    v = jnp.var(x, axis=axis, keepdims=True)
    return (x - m) / jnp.sqrt(v + eps)
def _scatter_add(tgt, idx, src, axis=0):
    return tgt.at[idx].add(src)
def _segment_sum(src, seg, n):
    return jax.ops.segment_sum(src, seg, n)
class _Rng:
    def __init__(self, key):
        self._k = key
    def _next(self):
        self._k, sub = jax.random.split(self._k)
        return sub
    def normal(self, shape):
        return jax.random.normal(self._next(), shape, dtype=jnp.bfloat16)
    def randint(self, lo, hi, shape):
        return jax.random.randint(self._next(), shape, lo, hi, dtype=jnp.int32)
    def uniform(self, shape, lo=0.0, hi=1.0):
        return jax.random.uniform(self._next(), shape, jnp.bfloat16, lo, hi)
    def permutation(self, n):
        return jax.random.permutation(self._next(), n)


kernel_name = 'parallel_sum__mha_block__swiglu_ffn__prompt'

def setup_inputs():
    _rng = _Rng(jax.random.key(int.from_bytes(__import__("os").urandom(4), "little")))
    _w = (lambda a: (lambda t: t.astype(jnp.bfloat16) if jnp.issubdtype(t.dtype, jnp.floating) else t)(jnp.asarray(a)))
    def _A_setup():
        B, S, D, H = 1, 2048, 640, 32
        return {
            "x": _w((lambda *s: _rng.normal(s) * 0.05)(B, S, D)),
            "wqkv": _w((lambda *s: _rng.normal(s) * 0.1)(D, 3 * D)),
            "wo": _w((lambda *s: _rng.normal(s) * 0.05)(D, D)),
        }
    _A_in = _A_setup()

    def _B_setup():
        B, S, D, F = 1, 2048, 640, 1536
        return {
            "x": _w((lambda *s: _rng.normal(s) * 0.05)(B, S, D)),
            "w_gate": _w((lambda *s: _rng.normal(s) * 0.05)(D, F)),
            "w_up": _w((lambda *s: _rng.normal(s) * 0.05)(D, F)),
            "w_down": _w((lambda *s: _rng.normal(s) * 0.05)(F, D)),
        }
    _B_in = _B_setup()

    return {
        "A_x": _A_in["x"],
        "A_wqkv": _A_in["wqkv"],
        "A_wo": _A_in["wo"],
        "B_x": _B_in["x"],
        "B_w_gate": _B_in["w_gate"],
        "B_w_up": _B_in["w_up"],
        "B_w_down": _B_in["w_down"],
    }

def reference(A_x, A_wqkv, A_wo, B_x, B_w_gate, B_w_up, B_w_down):
    def _A_ref(x, wqkv, wo):
        B, S, D = x.shape
        H = 32
        Dh = D // H
        qkv = (lambda x, *d: x.transpose(*d))((x @ wqkv).reshape(B, S, 3, H, Dh), 2, 0, 3, 1, 4)
        q, k, v = qkv[0], qkv[1], qkv[2]
        scores = jnp.einsum("bhqd,bhkd->bhqk", q, k) * (Dh ** -0.5)
        p = _softmax(scores, axis=-1)
        o = jnp.einsum("bhqk,bhkd->bhqd", p, v)
        return (lambda x, *d: x.transpose(*d))(o, 0, 2, 1, 3).reshape(B, S, D) @ wo

    def _B_ref(x, w_gate, w_up, w_down):
        g = _silu(x @ w_gate)
        u = x @ w_up
        return (g * u) @ w_down

    x = A_x
    xn = _layernorm(x, axis=-1)
    return x + _A_ref(xn, A_wqkv, A_wo) + _B_ref(xn, B_w_gate, B_w_up, B_w_down)
```

```python
import math

import jax
import jax.numpy as jnp
from jax import lax
import jax.experimental.pallas as pl
import jax.experimental.pallas.tpu as pltpu

_H = 32
_EPS = 1e-5
_LANES = 128
_BQ = 512
_CK = 128
_PAIRS = 1
_RP = 512
_RF = 512

_NN = (((1,), (0,)), ((), ()))
_NT = (((1,), (1,)), ((), ()))


def _dot(a, b, dims=_NN):
    return lax.dot_general(a, b, dims, preferred_element_type=jnp.float32)


def _pack(x):
    return pltpu.bitcast(x, jnp.uint32)


def _unpack(x):
    return pltpu.bitcast(x, jnp.bfloat16)


def _kernel(x_hbm, wqkv_hbm, wo_hbm, wg_hbm, wu_hbm, wd_hbm, out_hbm,
            x_v, wqkv_v, wo_v, wg_v, wu_v, wd_v, out_v,
            wqv_t, xn_v, k_v, qt_v, vt_v, ot_v, sa, sb,
            x_sem, w_sem, o_sem):
    S, D = x_v.shape
    dh = D // _H
    ng = D // _LANES
    half = _LANES // 2
    n_p, n_f, n_q = S // _RP, S // _RF, S // _BQ
    q_scale = dh ** -0.5 * math.log2(math.e)

    def x_copy(r):
        rows = pl.ds(r * _RP, _RP)
        return pltpu.make_async_copy(x_hbm.at[rows], x_v.at[rows], x_sem.at[r])

    w_copies = [
        pltpu.make_async_copy(src, dst, w_sem.at[i])
        for i, (src, dst) in enumerate((
            (wqkv_hbm, wqkv_v), (wg_hbm, wg_v), (wu_hbm, wu_v),
            (wd_hbm, wd_v), (wo_hbm, wo_v)))
    ]
    x_copy(0).start()
    w_copies[0].start()
    for r in range(1, n_p):
        x_copy(r).start()
    for c in w_copies[1:]:
        c.start()

    w_copies[0].wait()
    wqv_t[0:D // 2, :] = _pack(wqkv_v[:, 0:D].T)
    wqv_t[D // 2:D, :] = _pack(wqkv_v[:, 2 * D:3 * D].T)

    def project(r, carry):
        x_copy(r).wait()
        row0 = pl.multiple_of(r * _RP, _RP)
        word0 = pl.multiple_of(r * (_RP // 2), _RP // 2)
        cols = pl.ds(row0, _RP)
        x = x_v[cols, :].astype(jnp.float32)
        xc = x - jnp.mean(x, axis=-1, keepdims=True)
        var = jnp.mean(xc * xc, axis=-1, keepdims=True)
        xn = (xc * lax.rsqrt(var + _EPS)).astype(jnp.bfloat16)
        xn_v[pl.ds(word0, _RP // 2), :] = _pack(xn)

        k = _pack(_dot(xn, wqkv_v[:, D:2 * D]).astype(jnp.bfloat16))
        kg = [k[:, g * _LANES:(g + 1) * _LANES] for g in range(ng)]
        low = lax.broadcasted_iota(jnp.int32, kg[0].shape, 1) < half
        for g in range(ng):
            k_v[g, pl.ds(word0, _RP // 2), :] = kg[g]
        for g in range(ng - 1):
            k_v[ng + g, pl.ds(word0, _RP // 2), :] = jnp.where(
                low, kg[g + 1], kg[g])

        qv = _dot(_unpack(wqv_t[...]), xn, _NT)
        qt = _pack((qv[0:D] * q_scale).astype(jnp.bfloat16))
        hw = half // 2
        for g in range(ng):
            qt_v[g, :, cols] = qt[g * half:(g + 1) * half]
        for g in range(ng - 1):
            qt_v[ng + g, 0:hw, cols] = qt[(g + 1) * half:(g + 1) * half + hw]
            qt_v[ng + g, hw:half, cols] = qt[g * half + hw:(g + 1) * half]

        top = lax.broadcasted_iota(jnp.int32, (8, _RP), 0) < 4
        for p in range(_H // 2):
            v = qv[D + 2 * dh * p:D + 2 * dh * (p + 1)]
            vt_v[2 * p, 0:16, cols] = v[0:16]
            vt_v[2 * p, 16:24, cols] = jnp.where(top, v[16:24], 1.0)
            vt_v[2 * p + 1, 0:16, cols] = v[24:40]
            vt_v[2 * p + 1, 16:24, cols] = jnp.where(top, 1.0, v[16:24])
        return carry

    lax.fori_loop(0, n_p, project, 0)

    def masked_queries(h, qi):
        start = h * dh
        lo = start % _LANES
        g = start // _LANES + jnp.where(lo + dh > _LANES, ng, 0)
        q = qt_v[g, :, pl.ds(pl.multiple_of(qi * _BQ, _BQ), _BQ)]
        word = lax.broadcasted_iota(jnp.int32, q.shape, 0)
        keep = ((word - lo // 2) & (half - 1)) < dh // 2
        return g, _unpack(jnp.where(keep, q, jnp.zeros_like(q)))

    def stage(nxt, dst, cur, src, m, zero):
        if nxt is not None:
            g, q = masked_queries(*nxt)
        m_new = acc = None
        for c in range(S // _CK):
            if nxt is not None:
                k = _unpack(k_v[g, c * _CK // 2:(c + 1) * _CK // 2, :])
                s = _dot(k, q)
                dst[c * _CK:(c + 1) * _CK, :] = s
                cm = jnp.max(s.reshape(_CK // 8, 8, _BQ), axis=0)
                m_new = cm if m_new is None else jnp.maximum(m_new, cm)
            if cur is not None:
                rows = pl.ds(pl.multiple_of(zero + c * _CK, _CK), _CK)
                p = jnp.exp2(src[rows, :] - m).astype(jnp.bfloat16)
                o = _dot(vt_v[cur, :, c * _CK:(c + 1) * _CK], p)
                acc = o if acc is None else acc + o
        if nxt is not None:
            m_new = jnp.max(m_new, axis=0, keepdims=True)
        return m_new, acc

    n_units = (_H // 2) * n_q
    top = lax.broadcasted_iota(jnp.int32, (8, _BQ), 0) < 4

    def unit(u, m, zero, last=False):
        p, qi = u // n_q, u % n_q
        nxt = None if last else (2 * ((u + 1) // n_q), (u + 1) % n_q)
        m, even = stage((2 * p + 1, qi), sb, 2 * p, sa, m, zero)
        m, odd = stage(nxt, sa, 2 * p + 1, sb, m, zero)
        even = even * (1.0 / even[20:21])
        odd = odd * (1.0 / odd[16:17])
        o = jnp.concatenate(
            [even[0:16], jnp.where(top, even[16:24], odd[16:24]), odd[0:16]],
            axis=0)
        ot_v[pl.ds(pl.multiple_of(p * 2 * dh, 8), 2 * dh),
             pl.ds(pl.multiple_of(qi * _BQ, _BQ), _BQ)] = o
        return m

    def attend(i, m):
        zero = (i // n_units) * _CK
        for j in range(_PAIRS):
            m = unit(i * _PAIRS + j, m, zero)
        return m

    zero32 = jnp.int32(0)
    m, _ = stage((zero32, zero32), sa, None, None, None, None)
    n_iter = n_units // _PAIRS - 1
    m = lax.fori_loop(0, n_iter, attend, m)

    def tail(i, m):
        zero = (i // n_units) * _CK
        for j in range(_PAIRS):
            m_next = unit(i * _PAIRS + j, m, zero, last=j == _PAIRS - 1)
            m = m if m_next is None else m_next
        return m

    lax.fori_loop(n_iter, n_iter + 1, tail, m)

    for c in w_copies[1:]:
        c.wait()

    def out_copy(r):
        rows = pl.ds(r * _RF, _RF)
        return pltpu.make_async_copy(
            out_v.at[rows], out_hbm.at[rows], o_sem.at[r])

    def finish(r, carry):
        rows = pl.ds(pl.multiple_of(r * _RF, _RF), _RF)
        words = pl.ds(pl.multiple_of(r * (_RF // 2), _RF // 2), _RF // 2)
        xn = _unpack(xn_v[words, :])
        gate = _dot(xn, wg_v[...])
        up = _dot(xn, wu_v[...])
        hidden = (jax.nn.silu(gate) * up).astype(jnp.bfloat16)
        o = ot_v[:, rows].astype(jnp.bfloat16).T
        y = _dot(o, wo_v[...]) + _dot(hidden, wd_v[...])
        out_v[rows, :] = (x_v[rows, :].astype(jnp.float32) + y).astype(
            out_v.dtype)
        out_copy(r).start()
        return carry

    lax.fori_loop(0, n_f, finish, 0)
    for r in range(n_f):
        out_copy(r).wait()


@jax.jit
def pallas_parallel_sum__mha_block__swiglu_ffn__prompt_kernel(
    A_x: jax.Array,
    A_wqkv: jax.Array,
    A_wo: jax.Array,
    B_x: jax.Array,
    B_w_gate: jax.Array,
    B_w_up: jax.Array,
    B_w_down: jax.Array,
):
    del B_x
    B, S, D = A_x.shape
    F = B_w_gate.shape[1]
    assert B == 1 and D == 20 * _H and D % _LANES == 0
    ng = D // _LANES
    bf16, u32, f32 = jnp.bfloat16, jnp.uint32, jnp.float32
    hbm = pl.BlockSpec(memory_space=pl.ANY)

    out = pl.pallas_call(
        _kernel,
        in_specs=[hbm] * 6,
        out_specs=hbm,
        out_shape=jax.ShapeDtypeStruct((S, D), A_x.dtype),
        scratch_shapes=[
            pltpu.VMEM((S, D), bf16),
            pltpu.VMEM((D, 3 * D), bf16),
            pltpu.VMEM((D, D), bf16),
            pltpu.VMEM((D, F), bf16),
            pltpu.VMEM((D, F), bf16),
            pltpu.VMEM((F, D), bf16),
            pltpu.VMEM((S, D), A_x.dtype),
            pltpu.VMEM((D, D), u32),
            pltpu.VMEM((S // 2, D), u32),
            pltpu.VMEM((2 * ng - 1, S // 2, _LANES), u32),
            pltpu.VMEM((2 * ng - 1, _LANES // 2, S), u32),
            pltpu.VMEM((_H, 24, S), f32),
            pltpu.VMEM((D, S), f32),
            pltpu.VMEM((S, _BQ), f32),
            pltpu.VMEM((S, _BQ), f32),
            pltpu.SemaphoreType.DMA((S // _RP,)),
            pltpu.SemaphoreType.DMA((5,)),
            pltpu.SemaphoreType.DMA((S // _RF,)),
        ],
        compiler_params=pltpu.CompilerParams(
            vmem_limit_bytes=100 * 1024 * 1024),
        name="mha_swiglu",
    )(A_x.reshape(S, D), A_wqkv, A_wo, B_w_gate, B_w_up, B_w_down)
    return out.reshape(B, S, D)
```

```python
import math

import jax
import jax.numpy as jnp
from jax import lax
import jax.experimental.pallas as pl
import jax.experimental.pallas.tpu as pltpu

_H = 32
_DH = 20
_EPS = 1e-5
_LOG2E = math.log2(math.e)
_LANES = 128
_WIDE = 512
_BQ = _WIDE
_CK = 128
_RF = 256
_EARLY = 96
_EARLY_STEP = 16
_CHAINS = 2
_LATE = 208
_PARTS = 4
_SPLIT = 10

_NN = (((1,), (0,)), ((), ()))
_NT = (((1,), (1,)), ((), ()))


def _dot(a, b, dims=_NN):
    return lax.dot_general(a, b, dims, preferred_element_type=jnp.float32)


def _pack(x):
    return pltpu.bitcast(x.astype(jnp.bfloat16), jnp.uint32)


def _unpack(x):
    return pltpu.bitcast(x, jnp.bfloat16)


def _tile(i, size):
    return pl.ds(pl.multiple_of(i * size, size), size)


def _column_max(m):
    return jnp.broadcast_to(jnp.max(m, axis=0, keepdims=True), m.shape)


def _kernel(x_hbm, wqkv_hbm, wo_hbm, wg_hbm, wu_hbm, wd_hbm, out_hbm,
            x_v, wqkv_v, wo_v, wg_v, wu_v, wd_v, wqv_t, xn_v, k_v, kpair_v,
            kt_early, kt_late, qt_v, vt_v, ot_v, y_v, s_early, s_v, tables,
            zeros, x_sem, w_sem, o_sem):
    S, D = x_v.shape
    F = wg_v.shape[1]
    n_pairs, n_q, n_c = _H // 2, S // _BQ, S // _CK
    handed_out = [0]

    def zero():
        handed_out[0] += 1
        return zeros[handed_out[0] % zeros.shape[0]]

    def lay_out_keys(pairs, words):
        low = lax.broadcasted_iota(jnp.int32, (_BQ // 2, _LANES), 1) < _LANES // 2
        for p in pairs:
            g, lane = divmod(2 * _DH * p, _LANES)
            k = k_v[words, g * _LANES:(g + 1) * _LANES]
            if lane + 2 * _DH > _LANES:
                k = jnp.where(low, k_v[words, (g + 1) * _LANES:(g + 2) * _LANES], k)
            kpair_v[p, words, :] = pltpu.roll(k, _LANES - lane, 1) if lane else k

    def table_items(odd, p, qi):
        q_mxu, q_rows, k_cols = tables[odd]
        tile = qt_v.at[p, :, _tile(qi, _BQ)]

        def masked():
            q = tile[...]
            own = lax.broadcasted_iota(jnp.int32, q.shape, 0) < _DH
            if odd:
                q = jnp.concatenate(
                    [jnp.where(own, 0.0, q), jnp.zeros((8, _BQ), q.dtype)], axis=0)
            else:
                q = jnp.where(own, q, 0.0)[0:32]
            q_mxu[qi] = _pack(q)
            return lambda z: [
                pltpu.bitcast(q_mxu[qi + z, 0:8, 0:_LANES], jnp.float32)]

        def broadcasts(i):
            d = qi * (_DH // n_q) + i
            row = kt_late[pl.ds((2 * p + odd) * _DH + d, 1), :]
            col = jnp.broadcast_to(row, (_LANES, row.shape[1])).T[:_LATE]
            k_cols[:, d] = col.reshape(_LATE // 8, 8, _LANES)
            for e in range(i * n_q, (i + 1) * n_q):
                q_rows[qi, e] = jnp.broadcast_to(
                    tile[odd * _DH + e:odd * _DH + e + 1, :], (8, _BQ))
            return lambda z: [k_cols[z, d], q_rows[qi + z, e, :, 0:_LANES]]

        return [masked] + [lambda i=i: broadcasts(i) for i in range(_DH // n_q)]

    def value_items(odd, p, qi):
        z = zero()
        src, vt = s_v[odd].at[qi + z], vt_v.at[2 * p + odd + z]
        state = {}

        def item(c):
            if c == 0:
                early = jnp.concatenate(
                    [s_early[qi * (_BQ // _RF) + i, 2 * p + odd]
                     for i in range(_BQ // _RF)], axis=1)
                m = jnp.maximum(src[S:S + 8, :], early[_EARLY:])
                state["max"] = jnp.concatenate([m] * (_CK // 8), axis=0)
                s = jnp.concatenate([early[:_EARLY], src[_EARLY:_CK, :]], axis=0)
            else:
                s = src[c * _CK:(c + 1) * _CK, :]
            o = _dot(vt[:, c * _CK:(c + 1) * _CK], jnp.exp2(s - state["max"]))
            if c == 0:
                o = jnp.concatenate([jnp.where(z > 0, 0.0, o[:8]), o[8:]], axis=0)
            else:
                o = state["o"] + o
            state["o"] = o
            if c == n_c - 1:
                ot_v[2 * p + odd, :, _tile(qi, _BQ)] = o

        return [lambda c=c: item(c) for c in range(n_c)]

    def scores(odd, p, qi, values, side):
        q_mxu, q_rows, k_cols = tables[odd]
        dst = s_v[odd].at[qi]
        z = zero()
        never, keys, q = z > 0, kpair_v.at[p + z], _unpack(q_mxu[qi + z])
        q = jnp.concatenate(
            [q, jnp.zeros((_LANES - q.shape[0], _BQ), q.dtype)], axis=0)
        first = _EARLY + _LATE
        bounds = [first - 16 * (-c * (S - first) // 16 // n_c)
                  for c in range(n_c + 1)]
        n_parts, ticks = _LATE // 8 * _PARTS, (S - first) // 8 + len(values)
        state = dict(max=None, part=0, tick=2)

        def emit(row, s):
            dst[row:row + 8, :] = s
            m = state["max"]
            state["max"] = s if m is None else jnp.maximum(m, s)

        def tick():
            while state["part"] < min(n_parts, state["tick"] * n_parts // ticks):
                slab, part = divmod(state["part"], _PARTS)
                state["part"] += 1
                if part == 0:
                    state["z"], state["s"] = zero(), None
                rows = q_rows.at[qi + state["z"]]
                cols = k_cols.at[slab + state["z"]]
                for d in range(part * _DH // _PARTS, (part + 1) * _DH // _PARTS):
                    t = jnp.concatenate([cols[d]] * (_BQ // _LANES), axis=1) * rows[d]
                    state["s"] = t if d == 0 else state["s"] + t
                if part == _PARTS - 1:
                    emit(_EARLY + 8 * slab, state["s"])
                elif state["max"] is not None:
                    state["max"] = jnp.where(never, state["s"], state["max"])
            state["tick"] += 1

        for c in range(n_c):
            lo, hi = bounds[c], bounds[c + 1]
            s = _dot(_unpack(keys[lo // 2:hi // 2, :]), q)
            for row in range(lo, hi, 8):
                tick()
                emit(row, s[row - lo:row - lo + 8])
            if values:
                values[c]()
                tick()
            if c % 2 and 1 <= c // 2 <= len(side):
                m = [state["max"][:, i:i + _LANES] for i in range(0, _BQ, _LANES)]
                for i, written in enumerate(side[c // 2 - 1]()(zero())):
                    m[i] = jnp.where(never, written, m[i])
                state["max"] = jnp.concatenate(m, axis=1)
        assert state["part"] == n_parts
        dst[S:S + 8, :] = _column_max(state["max"])

    def first_head(qi, carry):
        scores(0, 0, qi, [], table_items(1, 0, qi))
        lay_out_keys(range(_SPLIT, n_pairs), _tile(qi, _BQ // 2))
        return carry

    def attend(h, carry):
        for odd in range(2):
            @pl.when(h % 2 == odd)
            def _():
                p = h // 2
                for qi in range(n_q):
                    scores(odd, p, qi, value_items(1 - odd, p + odd - 1, qi),
                           table_items(1 - odd, jnp.minimum(p + odd, n_pairs - 1), qi))
        return carry

    def early_keys(group, h):
        return s_v[group // n_q].at[group % n_q, _tile(h, _EARLY * _DH // n_q)]

    def early_slot(d, lo, hi):
        row, col = divmod(d, _BQ // _LANES)
        return (slice(row * _EARLY + lo, row * _EARLY + hi),
                slice(col * _LANES, (col + 1) * _LANES))

    def project(r, carry):
        cols, words = _tile(r, _BQ), _tile(r, _BQ // 2)
        lay_out_keys(range(_SPLIT), words)
        for d in range(_DH):
            row = kt_early[pl.ds(r * _DH + d, 1), :]
            col = jnp.broadcast_to(row, (_LANES, row.shape[1])).T
            for g in range(_H // n_q):
                early_keys(g, r)[early_slot(d, 0, _EARLY)] = col[
                    g * _EARLY:(g + 1) * _EARLY]
        qv = _dot(_unpack(wqv_t[...]), _unpack(xn_v[words, :]), _NT)
        q = qv[:D] * (_DH ** -0.5 * _LOG2E)
        top = lax.broadcasted_iota(jnp.int32, (8, _BQ), 0) < 4
        for p in range(n_pairs):
            qt_v[p, :, cols] = q[2 * _DH * p:2 * _DH * (p + 1)]
            v = qv[D + 2 * _DH * p:D + 2 * _DH * (p + 1)]
            vt_v[2 * p, 0:16, cols] = v[0:16]
            vt_v[2 * p, 16:24, cols] = jnp.where(top, v[16:24], 1.0)
            vt_v[2 * p + 1, 0:8, cols] = jnp.where(top, 1.0, v[16:24])
            vt_v[2 * p + 1, 8:24, cols] = v[24:40]
            if p == 0:
                for item in table_items(0, 0, r):
                    item()
        return carry

    def swiglu(r, carry):
        rows = _tile(r, _RF)
        xn = _unpack(xn_v[_tile(r, _RF // 2), :])
        never = zero() > 0
        n_t, n_step = _RF // _LANES, _EARLY // _EARLY_STEP
        n_units = _H * n_t * n_step
        ticks = 3 * (F // _LANES) * (D // _LANES) // 4 * (_RF // 8)
        state = dict(unit=0, tick=12)

        def early_scores(due):
            tile, step = divmod(state["unit"], n_step)
            h, t = divmod(tile, n_t)
            state["unit"] += 1
            if step == 0:
                q = qt_v[h // 2, :, _tile(r * n_t + t, _LANES)]
                state["q"] = [
                    jnp.broadcast_to(q[e:e + 1], (_EARLY_STEP, _LANES))
                    for e in range(h % 2 * _DH, (h % 2 + 1) * _DH)]
                state["k"] = early_keys(h // n_q, h % n_q + zero())
                state["max"] = jnp.full((8, _LANES), -jnp.inf, jnp.float32)
            lo, sums = step * _EARLY_STEP, []
            for d in range(_DH):
                v = state["k"][early_slot(d, lo, lo + _EARLY_STEP)] * state["q"][d]
                sums.append(v if d < _CHAINS else sums.pop(0) + v)
            s = sum(sums[1:], sums[0])
            dst = s_early.at[r, h, :, t * _LANES:(t + 1) * _LANES]
            dst[lo:lo + _EARLY_STEP, :] = s
            state["max"] = jnp.maximum(
                jnp.where(never, due, state["max"]),
                jnp.max(s.reshape(_EARLY_STEP // 8, 8, _LANES), axis=0))
            if step == n_step - 1:
                dst[_EARLY:, :] = _column_max(state["max"])

        def paced(y):
            for i in range(0, _RF, 8):
                state["tick"] += 1
                while state["unit"] < min(n_units, state["tick"] * n_units // ticks):
                    early_scores(y[i:i + 8, 0:_LANES])
            return y

        hidden = []
        for j in range(0, F, _WIDE // 2):
            both = slice(j, j + _WIDE // 2)
            rest = paced(_dot(xn[:, _WIDE:], jnp.concatenate(
                [wg_v[_WIDE:, both], wu_v[_WIDE:, both]], axis=1)))
            for i in range(0, _WIDE // 2, _LANES):
                gate, up = [
                    paced(_dot(xn[:, :_WIDE], w_v[:_WIDE, j + i:j + i + _LANES])
                          + rest[:, o + i:o + i + _LANES])
                    for o, w_v in ((0, wg_v), (_WIDE // 2, wu_v))]
                sigmoid = pltpu.reciprocal(
                    1.0 + jnp.exp2(gate * -_LOG2E), approx=True)
                hidden.append((gate * sigmoid * up).astype(jnp.bfloat16))
        hidden = jnp.concatenate(hidden, axis=1)
        for n in range(0, D, _LANES):
            y = x_v[rows, n:n + _LANES].astype(jnp.float32)
            for k in range(0, F, _WIDE):
                y = paced(y + _dot(hidden[:, k:k + _WIDE],
                                   wd_v[k:k + _WIDE, n:n + _LANES]))
            y_v[rows, n:n + _LANES] = y
        assert state["unit"] == n_units
        return carry

    col_groups = ((0, _WIDE), (_WIDE, D))

    def out_copy(r, i):
        lo, hi = col_groups[i]
        return pltpu.make_async_copy(
            x_v.at[_tile(r, _BQ), lo:hi], out_hbm.at[_tile(r, _BQ), lo:hi],
            o_sem.at[2 * r + i])

    def finish(r, carry):
        rows = _tile(r, _BQ)
        values = value_items(1, n_pairs - 1, r)
        top = lax.broadcasted_iota(jnp.int32, (8, _BQ), 0) < 4

        def normalized(pairs):
            o = []
            for p in pairs:
                even, odd = ot_v[2 * p, :, rows], ot_v[2 * p + 1, :, rows]
                even = even * (1.0 / even[_DH:_DH + 1])
                odd = odd * (1.0 / odd[0:1])
                o += [even[0:16], jnp.where(top, even[16:24], odd[0:8]), odd[8:24]]
            return o

        o = normalized(range(n_pairs - 1))
        lhs = jnp.concatenate(o, axis=0)[:_WIDE].astype(jnp.bfloat16).T
        y = []
        for i in range(_BQ // _LANES):
            row = []
            for n in range(0, D, _LANES):
                row.append(
                    _dot(lhs[i * _LANES:(i + 1) * _LANES], wo_v[:_WIDE, n:n + _LANES])
                    + y_v[_tile(r * (_BQ // _LANES) + i, _LANES), n:n + _LANES])
                for item in values[:2]:
                    item()
                values = values[2:]
            y.append(jnp.concatenate(row, axis=1))
        y = jnp.concatenate(y, axis=0)
        o += normalized([n_pairs - 1])
        lhs = jnp.concatenate(o, axis=0)[_WIDE:].astype(jnp.bfloat16).T
        for i, (lo, hi) in enumerate(col_groups):
            x_v[rows, lo:hi] = (
                y[:, lo:hi] + _dot(lhs, wo_v[_WIDE:, lo:hi])).astype(x_v.dtype)
            out_copy(r, i).start()
        return carry

    e, step = S // 8, 64
    x_copies = [
        pltpu.make_async_copy(x_hbm.at[lo:hi], x_v.at[lo:hi], x_sem.at[i])
        for i, (lo, hi) in enumerate(((0, 2 * e), (2 * e, 5 * e), (5 * e, S)))]
    wq_copy, wk_copy, wv_copy, *w_copies = [
        pltpu.make_async_copy(src, dst, w_sem.at[i])
        for i, (src, dst) in enumerate(
            [(wqkv_hbm.at[:, j:j + D], wqkv_v.at[:, j:j + D])
             for j in range(0, 3 * D, D)]
            + [(wg_hbm, wg_v), (wu_hbm, wu_v), (wd_hbm, wd_v), (wo_hbm, wo_v)])]

    def clear(i, carry):
        zeros[i] = 0
        return carry

    def layernorm(lo, hi):
        for r in range(lo, hi, step):
            x = x_v[r:r + step, :].astype(jnp.float32)
            xc = x - jnp.mean(x, axis=-1, keepdims=True)
            var = jnp.mean(xc * xc, axis=-1, keepdims=True)
            xn_v[r // 2:(r + step) // 2, :] = _pack(xc * lax.rsqrt(var + _EPS))

    def project_keys(lo, hi, rows, due=None):
        for r in range(lo, hi, rows):
            xn = xn_v[r // 2:(r + rows) // 2, :]
            if due is not None and r + rows == hi:
                z = zero()
                xn = jnp.concatenate(
                    [jnp.where(z > 0, due[_tile(z, 8), :], xn[:8]), xn[8:]], axis=0)
            k_v[r // 2:(r + rows) // 2, :] = _pack(
                _dot(_unpack(xn), wqkv_v[:, D:2 * D]))

    x_copies[0].start()
    wk_copy.start()
    lax.fori_loop(0, zeros.shape[0], clear, 0)
    x_copies[0].wait()
    x_copies[1].start()
    layernorm(0, 2 * e)
    wk_copy.wait()
    x_copies[2].start()
    project_keys(0, e, e)
    x_copies[1].wait()
    wq_copy.start()
    wv_copy.start()
    project_keys(e, 2 * e, e)
    layernorm(2 * e, 5 * e)
    project_keys(2 * e, 5 * e - step, step)
    for copy in (x_copies[2], wq_copy, wv_copy):
        copy.wait()
    for copy in w_copies:
        copy.start()
    project_keys(5 * e - step, 5 * e, step)
    layernorm(5 * e, S)
    kt = _unpack(k_v[0:_LANES // 2, :]).T.astype(jnp.float32)
    kt_early[...] = jnp.concatenate(
        [kt[g:g + n_q * _DH, :_EARLY] for g in range(0, D, n_q * _DH)], axis=1)
    kt_late[...] = _unpack(
        k_v[_EARLY // 2:(_EARLY + kt_late.shape[1]) // 2, :]).T.astype(jnp.float32)
    wqv_t[:D // 2, :] = _pack(wqkv_v[:, :D].T)
    wqv_t[D // 2:, :] = _pack(wqkv_v[:, 2 * D:].T)
    project_keys(5 * e, S, step, due=wqv_t)

    lax.fori_loop(0, n_q, project, 0)
    for copy in w_copies:
        copy.wait()
    lax.fori_loop(0, S // _RF, swiglu, 0)
    lax.fori_loop(0, n_q, first_head, 0)
    lax.fori_loop(1, _H, attend, 0)
    lax.fori_loop(0, n_q, finish, 0)
    for r in range(n_q):
        for i in range(len(col_groups)):
            out_copy(r, i).wait()


@jax.jit
def pallas_parallel_sum__mha_block__swiglu_ffn__prompt_kernel(
    A_x: jax.Array,
    A_wqkv: jax.Array,
    A_wo: jax.Array,
    B_x: jax.Array,
    B_w_gate: jax.Array,
    B_w_up: jax.Array,
    B_w_down: jax.Array,
):
    del B_x
    B, S, D = A_x.shape
    assert B == 1 and S == 4 * _BQ and D == _DH * _H
    u32, f32 = jnp.uint32, jnp.float32
    n_q = S // _BQ
    operands = (A_x.reshape(S, D), A_wqkv, A_wo, B_w_gate, B_w_up, B_w_down)
    hbm = pl.BlockSpec(memory_space=pl.ANY)

    def tables(words):
        return (pltpu.VMEM((n_q, words, _BQ), u32),
                pltpu.VMEM((n_q, _DH, 8, _BQ), f32),
                pltpu.VMEM((_LATE // 8, _DH, 8, _LANES), f32))

    out = pl.pallas_call(
        _kernel,
        in_specs=[hbm] * len(operands),
        out_specs=hbm,
        out_shape=jax.ShapeDtypeStruct((S, D), A_x.dtype),
        scratch_shapes=[
            *[pltpu.VMEM(a.shape, a.dtype) for a in operands],
            pltpu.VMEM((D, D), u32),
            pltpu.VMEM((S // 2, D), u32),
            pltpu.VMEM((S // 2, D), u32),
            pltpu.VMEM((_H // 2, S // 2, _LANES), u32),
            pltpu.VMEM((n_q * _DH, _H // n_q * _EARLY), f32),
            pltpu.VMEM((D, pl.cdiv(_LATE, _LANES) * _LANES), f32),
            pltpu.VMEM((_H // 2, 2 * _DH, S), f32),
            pltpu.VMEM((_H, 24, S), f32),
            pltpu.VMEM((_H, 24, S), f32),
            pltpu.VMEM((S, D), f32),
            pltpu.VMEM((S // _RF, _H, _EARLY + 8, _RF), f32),
            (pltpu.VMEM((n_q, S + 8, _BQ), f32),) * 2,
            (tables(16), tables(24)),
            pltpu.SMEM((n_q * (_LATE // 8 + 8),), jnp.int32),
            pltpu.SemaphoreType.DMA((3,)),
            pltpu.SemaphoreType.DMA((7,)),
            pltpu.SemaphoreType.DMA((2 * n_q,)),
        ],
        compiler_params=pltpu.CompilerParams(
            vmem_limit_bytes=122 * 1024 * 1024),
        name="mha_swiglu",
    )(*operands)
    return out.reshape(B, S, D)
```
